```python
import jax
import jax.numpy as jnp

def _softmax(x, axis=-1):
    return jax.nn.softmax(x, axis=axis)
def _gelu(x):
    return jax.nn.gelu(x, approximate=True)
def _silu(x):
    return jax.nn.silu(x)
def _sigmoid(x):
    return jax.nn.sigmoid(x)
def _layernorm(x, axis=-1, eps=1e-5):
    m = jnp.mean(x, axis=axis, keepdims=True)
    v = jnp.var(x, axis=axis, keepdims=True)
    return (x - m) / jnp.sqrt(v + eps)
def _scatter_add(tgt, idx, src, axis=0):
    return tgt.at[idx].add(src)
def _segment_sum(src, seg, n):
    return jax.ops.segment_sum(src, seg, n)
class _Rng:
    def __init__(self, key):
        self._k = key
    def _next(self):
        self._k, sub = jax.random.split(self._k)
        return sub
    def normal(self, shape):
        return jax.random.normal(self._next(), shape, dtype=jnp.bfloat16)
    def randint(self, lo, hi, shape):
        return jax.random.randint(self._next(), shape, lo, hi, dtype=jnp.int32)
    def uniform(self, shape, lo=0.0, hi=1.0):
        return jax.random.uniform(self._next(), shape, jnp.bfloat16, lo, hi)
    def permutation(self, n):
        return jax.random.permutation(self._next(), n)


kernel_name = 'concat_heads__gqa_block_cached__compressed_kv_cla__decode'

def setup_inputs():
    _rng = _Rng(jax.random.key(int.from_bytes(__import__("os").urandom(4), "little")))
    _w = (lambda a: (lambda t: t.astype(jnp.bfloat16) if jnp.issubdtype(t.dtype, jnp.floating) else t)(jnp.asarray(a)))
    def _A_setup():
        B, Sq, D = 2, 1, 512
        Hq, Hkv, Sk, Dh = 32, 32, 8192, 128
        assert Hq % Hkv == 0, (Hq, Hkv)
        return {
            "x": _w((lambda *s: _rng.normal(s) * 0.05)(B, Sq, D)),
            "k_cache": _w((lambda *s: _rng.normal(s) * 0.05)(B, Hkv, Sk, Dh)),
            "v_cache": _w((lambda *s: _rng.normal(s) * 0.05)(B, Hkv, Sk, Dh)),
            "wq": _w((lambda *s: _rng.normal(s) * 0.05)(D, Hq * Dh) * (D ** -0.5)),
            "wo": _w((lambda *s: _rng.normal(s) * 0.05)(Hq * Dh, D) * ((Hq * Dh) ** -0.5)),
        }
    _A_in = _A_setup()

    def _B_setup():
        B, H, Sq, Sk, D, M = 2, 32, 1, 8192, 128, 512
        Dc = 4 * D
        return {
            "x": _w((lambda *s: _rng.normal(s) * 0.05)(B, Sq, M)),
            "c_kv": _w((lambda *s: _rng.normal(s) * 0.05)(B, Sk, Dc)),
            "w_q": _w((lambda *s: _rng.normal(s) * 0.05)(M, H, D) * (M ** -0.5)),
            "w_uk": _w((lambda *s: _rng.normal(s) * 0.05)(Dc, H, D) * (Dc ** -0.5)),
            "w_uv": _w((lambda *s: _rng.normal(s) * 0.05)(Dc, H, D) * (Dc ** -0.5)),
            "w_o": _w((lambda *s: _rng.normal(s) * 0.05)(H, D, M) * ((H * D) ** -0.5)),
        }
    _B_in = _B_setup()

    return {
        "A_x": _A_in["x"],
        "A_k_cache": _A_in["k_cache"],
        "A_v_cache": _A_in["v_cache"],
        "A_wq": _A_in["wq"],
        "A_wo": _A_in["wo"],
        "B_x": _B_in["x"],
        "B_c_kv": _B_in["c_kv"],
        "B_w_q": _B_in["w_q"],
        "B_w_uk": _B_in["w_uk"],
        "B_w_uv": _B_in["w_uv"],
        "B_w_o": _B_in["w_o"],
    }

def reference(A_x, A_k_cache, A_v_cache, A_wq, A_wo, B_x, B_c_kv, B_w_q, B_w_uk, B_w_uv, B_w_o):
    def _A_ref(x, k_cache, v_cache, wq, wo):
        B, Sq, D = x.shape
        Hq, Dh = 32, 128
        Hkv = k_cache.shape[1]
        rep = Hq // Hkv
        q = (lambda x, *d: x.transpose(*d))((x @ wq).reshape(B, Sq, Hq, Dh), 0, 2, 1, 3)
        k = jnp.repeat(k_cache, rep, axis=1)
        v = jnp.repeat(v_cache, rep, axis=1)
        scores = jnp.einsum("bhqd,bhkd->bhqk", q, k) * (Dh ** -0.5)
        p = _softmax(scores, axis=-1)
        o = jnp.einsum("bhqk,bhkd->bhqd", p, v)
        return (lambda x, *d: x.transpose(*d))(o, 0, 2, 1, 3).reshape(B, Sq, Hq * Dh) @ wo

    def _B_ref(x, c_kv, w_q, w_uk, w_uv, w_o):
        B, Sq, M = x.shape[0], x.shape[1], x.shape[2]
        Sk = c_kv.shape[1]
        H, D = w_q.shape[1], w_q.shape[2]
        q = jnp.einsum("bqm,mhd->bhqd", x, w_q)
        k = jnp.einsum("bkc,chd->bhkd", c_kv, w_uk)
        v = jnp.einsum("bkc,chd->bhkd", c_kv, w_uv)
        scores = jnp.einsum("bhqd,bhkd->bhqk", q, k) * (D ** -0.5)
        off = Sk - Sq
        qi = jnp.arange(Sq)[:, None]
        kj = jnp.arange(Sk)[None, :]
        cmask = kj <= (qi + off)
        scores = jnp.where(cmask[None, None], scores, -1e9)
        p = _softmax(scores, axis=-1)
        ctx = jnp.einsum("bhqk,bhkd->bhqd", p, v)
        return jnp.einsum("bhqd,hdm->bqm", ctx, w_o)

    a = _A_ref(A_x, A_k_cache, A_v_cache, A_wq, A_wo)
    b = _B_ref(B_x, B_c_kv, B_w_q, B_w_uk, B_w_uv, B_w_o)
    return jnp.concatenate([a, b], axis=-1)
```

```python
import jax
import jax.numpy as jnp
from jax import lax
import jax.experimental.pallas as pl
import jax.experimental.pallas.tpu as pltpu

F32 = jnp.float32
BF16 = jnp.bfloat16

B = 2
H = 32
S = 8192
DH = 128
DM = 512
DC = 512
BH = B * H

NSLOT = 4
NCH = 4
CH = S // NCH
NCKV = 4
CKV = S // NCKV

NN = (((1,), (0,)), ((), ()))
NT = (((1,), (1,)), ((), ()))


def _dot(a, b, dims=NN):
    return lax.dot_general(a, b, dims, preferred_element_type=F32)


def _iota(shape, dim):
    return lax.broadcasted_iota(jnp.int32, shape, dim)


def _kernel(xa_hbm, k_hbm, v_hbm, wq_hbm, wo_hbm,
            xb_hbm, ckv_hbm, wqb_hbm, wuk_hbm, wuv_hbm, wob_hbm,
            out_ref,
            xa_v, xb_v, wq_v, wo_v, ckv_v, wqb_v, wuk_v, wuv_v, wob_v,
            kbuf, vbuf, q_scr, e0_scr,
            wsem, csem, ksem, vsem):
    def wcopy(i, src, dst):
        return pltpu.make_async_copy(src, dst, wsem.at[i])

    cp_xa = wcopy(0, xa_hbm, xa_v)
    cp_xb = wcopy(1, xb_hbm, xb_v)
    cp_wq = wcopy(2, wq_hbm, wq_v)
    cp_wqb = wcopy(3, wqb_hbm, wqb_v)
    cp_wuk = wcopy(4, wuk_hbm, wuk_v)
    cp_wuv = wcopy(5, wuv_hbm, wuv_v)
    cp_wob = wcopy(6, wob_hbm, wob_v)
    cp_wo = wcopy(7, wo_hbm, wo_v)

    def ckv_copy(b, c):
        return pltpu.make_async_copy(ckv_hbm.at[b, pl.ds(c * CKV, CKV)],
                                     ckv_v.at[b, pl.ds(c * CKV, CKV)],
                                     csem.at[b * NCKV + c])

    def kv_copies(src, buf, sem, i, slot):
        return [pltpu.make_async_copy(src.at[pl.ds(i * S + c * CH, CH)],
                                      buf.at[slot, pl.ds(c * CH, CH)],
                                      sem.at[slot * NCH + c]) for c in range(NCH)]

    def start_k(i, slot):
        for cp in kv_copies(k_hbm, kbuf, ksem, i, slot):
            cp.start()

    def start_v(i, slot):
        for cp in kv_copies(v_hbm, vbuf, vsem, i, slot):
            cp.start()

    cp_xa.start()
    cp_xb.start()
    cp_wq.start()
    cp_wqb.start()
    cp_wuk.start()
    for b in range(B):
        for c in range(NCKV):
            ckv_copy(b, c).start()
    cp_wuv.start()
    cp_wob.start()
    cp_wo.start()
    for s in range(NSLOT):
        start_k(s, s)
        start_v(s, s)

    e0_scr[...] = (_iota((128, 128 * H), 1) // H == _iota((128, 128 * H), 0)).astype(BF16)
    head_mask = (_iota((BH, 128), 1) % H) == (_iota((BH, 128), 0) % H)

    def mask_heads(t):
        return jnp.concatenate(
            [jnp.where(head_mask, t[:, j * 128:(j + 1) * 128], 0.0).astype(BF16)
             for j in range(t.shape[1] // 128)], axis=1)

    def expand_contract(lmat, w_ref):
        acc = jnp.zeros((BH, DH), F32)
        for u in range(lmat.shape[1] // 128):
            lx = mask_heads(_dot(lmat[:, u * 128:(u + 1) * 128], e0_scr[...]))
            acc = acc + _dot(lx, w_ref[pl.ds(u * 128 * H, 128 * H), :])
        return acc

    def contract_compress(q, w_ref):
        outs = []
        for u in range(w_ref.shape[0] // (128 * H)):
            t = mask_heads(_dot(q, w_ref[pl.ds(u * 128 * H, 128 * H), :], NT))
            outs.append(_dot(t, e0_scr[...], NT))
        return jnp.concatenate(outs, axis=1)

    cp_xa.wait()
    cp_wq.wait()
    xa = xa_v[...].reshape(B, DM)
    xa8 = jnp.concatenate([xa, jnp.zeros((16 - B, DM), BF16)], axis=0)
    qa = _dot(xa8, wq_v[...]).astype(BF16).astype(F32)
    for b in range(B):
        for h in range(H):
            q_scr[pl.ds(b * H + h, 1), :] = qa[b:b + 1, h * DH:(h + 1) * DH]

    cp_xb.wait()
    xb = xb_v[...].reshape(B, DM)
    xb_rows = jnp.concatenate(
        [jnp.broadcast_to(xb[b:b + 1, :], (H, DM)) for b in range(B)], axis=0)
    cp_wqb.wait()
    qb = expand_contract(xb_rows, wqb_v).astype(BF16)
    cp_wuk.wait()
    q_lat = contract_compress(qb, wuk_v).astype(BF16)

    ctx_lat = []
    for b in range(B):
        ql = q_lat[b * H:(b + 1) * H, :]
        ss = []
        for c in range(NCKV):
            ckv_copy(b, c).wait()
            ss.append(_dot(ql, ckv_v[b, pl.ds(c * CKV, CKV), :], NT))
        s = jnp.concatenate(ss, axis=1) * (DH ** -0.5)
        m = jnp.max(s, axis=1, keepdims=True)
        p = jnp.exp(s - m)
        l = jnp.sum(p, axis=1, keepdims=True)
        o = _dot(p.astype(BF16), ckv_v[b])
        ctx_lat.append(o / l)
    ctx_lat = jnp.concatenate(ctx_lat, axis=0).astype(BF16)

    cp_wuv.wait()
    ctx = expand_contract(ctx_lat, wuv_v).astype(BF16)
    ctx2 = jnp.concatenate(
        [jnp.concatenate([ctx[b * H + h:b * H + h + 1, :] for h in range(H)], axis=1)
         for b in range(B)] + [jnp.zeros((16 - B, H * DH), BF16)], axis=0)
    cp_wob.wait()
    out_b = _dot(ctx2, wob_v[...])
    for b in range(B):
        out_ref[b, :, DM:2 * DM] = out_b[b:b + 1, :].astype(out_ref.dtype)

    cp_wo.wait()

    def head_step(i, acc):
        slot = i % NSLOT
        nxt = i + NSLOT
        q = jnp.broadcast_to(q_scr[pl.ds(i, 1), :], (16, DH)).astype(BF16)
        ss = []
        kc = kv_copies(k_hbm, kbuf, ksem, i, slot)
        for c in range(NCH):
            kc[c].wait()
            ss.append(_dot(q, kbuf[slot, pl.ds(c * CH, CH), :], NT)[0:8])
        s = jnp.concatenate(ss, axis=1) * (DH ** -0.5)

        @pl.when(nxt < BH)
        def _():
            start_k(nxt, slot)

        m = jnp.max(s, axis=1, keepdims=True)
        p = jnp.exp(s - m)
        l = jnp.sum(p, axis=1, keepdims=True)
        pb = jnp.concatenate([p, p], axis=0).astype(BF16)
        o = jnp.zeros((16, DH), F32)
        vc = kv_copies(v_hbm, vbuf, vsem, i, slot)
        for c in range(NCH):
            vc[c].wait()
            o = o + _dot(pb[:, c * CH:(c + 1) * CH], vbuf[slot, pl.ds(c * CH, CH), :])

        @pl.when(nxt < BH)
        def _():
            start_v(nxt, slot)

        o = (o[0:8] / l)
        ob = jnp.concatenate([o, o], axis=0).astype(BF16)
        h = i % H
        return acc + _dot(ob, wo_v[pl.ds(pl.multiple_of(h * DH, DH), DH), :])[0:8]

    for b in range(B):
        acc = lax.fori_loop(b * H, (b + 1) * H, head_step, jnp.zeros((8, DM), F32))
        out_ref[b, :, 0:DM] = acc[0:1, :].astype(out_ref.dtype)


@jax.jit
def pallas_concat_heads__gqa_block_cached__compressed_kv_cla__decode_kernel(
    A_x: jax.Array,
    A_k_cache: jax.Array,
    A_v_cache: jax.Array,
    A_wq: jax.Array,
    A_wo: jax.Array,
    B_x: jax.Array,
    B_c_kv: jax.Array,
    B_w_q: jax.Array,
    B_w_uk: jax.Array,
    B_w_uv: jax.Array,
    B_w_o: jax.Array,
):
    any_spec = pl.BlockSpec(memory_space=pl.ANY)
    scratch = [
        pltpu.VMEM((B, 1, DM), BF16),
        pltpu.VMEM((B, 1, DM), BF16),
        pltpu.VMEM((DM, H * DH), BF16),
        pltpu.VMEM((H * DH, DM), BF16),
        pltpu.VMEM((B, S, DC), BF16),
        pltpu.VMEM((DM * H, DH), BF16),
        pltpu.VMEM((DC * H, DH), BF16),
        pltpu.VMEM((DC * H, DH), BF16),
        pltpu.VMEM((H * DH, DM), BF16),
        pltpu.VMEM((NSLOT, S, DH), BF16),
        pltpu.VMEM((NSLOT, S, DH), BF16),
        pltpu.VMEM((BH, DH), F32),
        pltpu.VMEM((128, 128 * H), BF16),
        pltpu.SemaphoreType.DMA((8,)),
        pltpu.SemaphoreType.DMA((B * NCKV,)),
        pltpu.SemaphoreType.DMA((NSLOT * NCH,)),
        pltpu.SemaphoreType.DMA((NSLOT * NCH,)),
    ]
    return pl.pallas_call(
        _kernel,
        out_shape=jax.ShapeDtypeStruct((B, 1, 2 * DM), BF16),
        in_specs=[any_spec] * 11,
        out_specs=pl.BlockSpec(memory_space=pltpu.VMEM),
        scratch_shapes=scratch,
        compiler_params=pltpu.CompilerParams(vmem_limit_bytes=100 * 1024 * 1024),
    )(
        A_x,
        A_k_cache.reshape(B * H * S, DH),
        A_v_cache.reshape(B * H * S, DH),
        A_wq,
        A_wo,
        B_x,
        B_c_kv,
        B_w_q.reshape(DM * H, DH),
        B_w_uk.reshape(DC * H, DH),
        B_w_uv.reshape(DC * H, DH),
        B_w_o.reshape(H * DH, DM),
    )
```

```python
import jax
import jax.numpy as jnp
from jax import lax
import jax.experimental.pallas as pl
import jax.experimental.pallas.tpu as pltpu

F32 = jnp.float32
BF16 = jnp.bfloat16

B = 2
H = 32
S = 8192
DH = 128
DM = 512
DC = 512
BH = B * H

NSLOT = 4
NCH = 4
CH = S // NCH
NCKV = 4
CKV = S // NCKV

NN = (((1,), (0,)), ((), ()))
NT = (((1,), (1,)), ((), ()))


def _dot(a, b, dims=NN):
    return lax.dot_general(a, b, dims, preferred_element_type=F32)


def _iota(shape, dim):
    return lax.broadcasted_iota(jnp.int32, shape, dim)


def _kernel(xa_hbm, k_hbm, v_hbm, wq_hbm, wo_hbm,
            xb_hbm, ckv_hbm, wqb_hbm, wuk_hbm, wuv_hbm, wob_hbm,
            out_ref,
            xa_v, xb_v, wq_v, wo_v, ckv_v, wqb_v, wuk_v, wuv_v, wob_v,
            kbuf, vbuf, q_scr, e0_scr,
            wsem, csem, ksem, vsem):
    def wcopy(i, src, dst):
        return pltpu.make_async_copy(src, dst, wsem.at[i])

    cp_xa = wcopy(0, xa_hbm, xa_v)
    cp_xb = wcopy(1, xb_hbm, xb_v)
    cp_wq = wcopy(2, wq_hbm, wq_v)
    cp_wqb = wcopy(3, wqb_hbm, wqb_v)
    cp_wuk = wcopy(4, wuk_hbm, wuk_v)
    cp_wuv = wcopy(5, wuv_hbm, wuv_v)
    cp_wob = wcopy(6, wob_hbm, wob_v)
    cp_wo = wcopy(7, wo_hbm, wo_v)

    def ckv_copy(b, c):
        return pltpu.make_async_copy(ckv_hbm.at[b, pl.ds(c * CKV, CKV)],
                                     ckv_v.at[b, pl.ds(c * CKV, CKV)],
                                     csem.at[b * NCKV + c])

    def kv_copies(src, buf, sem, i, slot):
        return [pltpu.make_async_copy(src.at[pl.ds(i * S + c * CH, CH)],
                                      buf.at[slot, pl.ds(c * CH, CH)],
                                      sem.at[slot * NCH + c]) for c in range(NCH)]

    def start_k(i, slot):
        for cp in kv_copies(k_hbm, kbuf, ksem, i, slot):
            cp.start()

    def start_v(i, slot):
        for cp in kv_copies(v_hbm, vbuf, vsem, i, slot):
            cp.start()

    cp_xa.start()
    cp_xb.start()
    cp_wq.start()
    cp_wqb.start()
    cp_wuk.start()
    for b in range(B):
        for c in range(NCKV):
            ckv_copy(b, c).start()
    cp_wuv.start()
    cp_wob.start()
    cp_wo.start()
    for s in range(NSLOT):
        start_k(s, s)
        start_v(s, s)

    e0_scr[...] = (_iota((128, 128 * H), 1) // H == _iota((128, 128 * H), 0)).astype(BF16)
    head_mask = (_iota((BH, 128), 1) % H) == (_iota((BH, 128), 0) % H)

    def mask_heads(t):
        return jnp.concatenate(
            [jnp.where(head_mask, t[:, j * 128:(j + 1) * 128], 0.0).astype(BF16)
             for j in range(t.shape[1] // 128)], axis=1)

    def expand_contract(lmat, w_ref):
        acc = jnp.zeros((BH, DH), F32)
        for u in range(lmat.shape[1] // 128):
            lx = mask_heads(_dot(lmat[:, u * 128:(u + 1) * 128], e0_scr[...]))
            acc = acc + _dot(lx, w_ref[pl.ds(u * 128 * H, 128 * H), :])
        return acc

    def contract_compress(q, w_ref):
        outs = []
        for u in range(w_ref.shape[0] // (128 * H)):
            t = mask_heads(_dot(q, w_ref[pl.ds(u * 128 * H, 128 * H), :], NT))
            outs.append(_dot(t, e0_scr[...], NT))
        return jnp.concatenate(outs, axis=1)

    cp_xa.wait()
    cp_wq.wait()
    xa = xa_v[...]
    xa8 = jnp.concatenate([xa, jnp.zeros((16 - B, DM), BF16)], axis=0)
    qa = _dot(xa8, wq_v[...]).astype(BF16).astype(F32)
    for b in range(B):
        for h in range(H):
            q_scr[pl.ds(b * H + h, 1), :] = qa[b:b + 1, h * DH:(h + 1) * DH]

    cp_xb.wait()
    xb = xb_v[...]
    xb_rows = jnp.concatenate(
        [jnp.broadcast_to(xb[b:b + 1, :], (H, DM)) for b in range(B)], axis=0)
    cp_wqb.wait()
    qb = expand_contract(xb_rows, wqb_v).astype(BF16)
    cp_wuk.wait()
    q_lat = contract_compress(qb, wuk_v).astype(BF16)

    ctx_lat = []
    for b in range(B):
        ql = q_lat[b * H:(b + 1) * H, :]
        ss = []
        for c in range(NCKV):
            ckv_copy(b, c).wait()
            ss.append(_dot(ql, ckv_v[b, pl.ds(c * CKV, CKV), :], NT))
        s = jnp.concatenate(ss, axis=1) * (DH ** -0.5)
        m = jnp.max(s, axis=1, keepdims=True)
        p = jnp.exp(s - m)
        l = jnp.sum(p, axis=1, keepdims=True)
        o = _dot(p.astype(BF16), ckv_v[b])
        ctx_lat.append(o / l)
    ctx_lat = jnp.concatenate(ctx_lat, axis=0).astype(BF16)

    cp_wuv.wait()
    ctx = expand_contract(ctx_lat, wuv_v).astype(BF16)
    ctx2 = jnp.concatenate(
        [jnp.concatenate([ctx[b * H + h:b * H + h + 1, :] for h in range(H)], axis=1)
         for b in range(B)] + [jnp.zeros((16 - B, H * DH), BF16)], axis=0)
    cp_wob.wait()
    out_b = _dot(ctx2, wob_v[...])
    for b in range(B):
        out_ref[b:b + 1, DM:2 * DM] = out_b[b:b + 1, :].astype(out_ref.dtype)

    cp_wo.wait()

    def head_step(i, acc):
        slot = i % NSLOT
        nxt = i + NSLOT
        q = jnp.broadcast_to(q_scr[pl.ds(i, 1), :], (16, DH)).astype(BF16)
        ss = []
        kc = kv_copies(k_hbm, kbuf, ksem, i, slot)
        for c in range(NCH):
            kc[c].wait()
            ss.append(_dot(q, kbuf[slot, pl.ds(c * CH, CH), :], NT)[0:8])
        s = jnp.concatenate(ss, axis=1) * (DH ** -0.5)

        @pl.when(nxt < BH)
        def _():
            start_k(nxt, slot)

        m = jnp.max(s, axis=1, keepdims=True)
        p = jnp.exp(s - m)
        l = jnp.sum(p, axis=1, keepdims=True)
        pb = jnp.concatenate([p, p], axis=0).astype(BF16)
        o = jnp.zeros((16, DH), F32)
        vc = kv_copies(v_hbm, vbuf, vsem, i, slot)
        for c in range(NCH):
            vc[c].wait()
            o = o + _dot(pb[:, c * CH:(c + 1) * CH], vbuf[slot, pl.ds(c * CH, CH), :])

        @pl.when(nxt < BH)
        def _():
            start_v(nxt, slot)

        o = (o[0:8] / l)
        ob = jnp.concatenate([o, o], axis=0).astype(BF16)
        h = i % H
        return acc + _dot(ob, wo_v[pl.ds(pl.multiple_of(h * DH, DH), DH), :])[0:8]

    for b in range(B):
        acc = lax.fori_loop(b * H, (b + 1) * H, head_step, jnp.zeros((8, DM), F32))
        out_ref[b:b + 1, 0:DM] = acc[0:1, :].astype(out_ref.dtype)


@jax.jit
def pallas_concat_heads__gqa_block_cached__compressed_kv_cla__decode_kernel(
    A_x: jax.Array,
    A_k_cache: jax.Array,
    A_v_cache: jax.Array,
    A_wq: jax.Array,
    A_wo: jax.Array,
    B_x: jax.Array,
    B_c_kv: jax.Array,
    B_w_q: jax.Array,
    B_w_uk: jax.Array,
    B_w_uv: jax.Array,
    B_w_o: jax.Array,
):
    any_spec = pl.BlockSpec(memory_space=pl.ANY)
    scratch = [
        pltpu.VMEM((B, DM), BF16),
        pltpu.VMEM((B, DM), BF16),
        pltpu.VMEM((DM, H * DH), BF16),
        pltpu.VMEM((H * DH, DM), BF16),
        pltpu.VMEM((B, S, DC), BF16),
        pltpu.VMEM((DM * H, DH), BF16),
        pltpu.VMEM((DC * H, DH), BF16),
        pltpu.VMEM((DC * H, DH), BF16),
        pltpu.VMEM((H * DH, DM), BF16),
        pltpu.VMEM((NSLOT, S, DH), BF16),
        pltpu.VMEM((NSLOT, S, DH), BF16),
        pltpu.VMEM((BH, DH), F32),
        pltpu.VMEM((128, 128 * H), BF16),
        pltpu.SemaphoreType.DMA((8,)),
        pltpu.SemaphoreType.DMA((B * NCKV,)),
        pltpu.SemaphoreType.DMA((NSLOT * NCH,)),
        pltpu.SemaphoreType.DMA((NSLOT * NCH,)),
    ]
    out = pl.pallas_call(
        _kernel,
        out_shape=jax.ShapeDtypeStruct((B, 2 * DM), BF16),
        in_specs=[any_spec] * 11,
        out_specs=pl.BlockSpec(memory_space=pltpu.VMEM),
        scratch_shapes=scratch,
        compiler_params=pltpu.CompilerParams(vmem_limit_bytes=100 * 1024 * 1024),
    )(
        A_x.reshape(B, DM),
        A_k_cache.reshape(B * H * S, DH),
        A_v_cache.reshape(B * H * S, DH),
        A_wq,
        A_wo,
        B_x.reshape(B, DM),
        B_c_kv,
        B_w_q.reshape(DM * H, DH),
        B_w_uk.reshape(DC * H, DH),
        B_w_uv.reshape(DC * H, DH),
        B_w_o.reshape(H * DH, DM),
    )
    return out.reshape(B, 1, 2 * DM)
```

```python
import jax
import jax.numpy as jnp
from jax import lax
import jax.experimental.pallas as pl
import jax.experimental.pallas.tpu as pltpu

F32 = jnp.float32
BF16 = jnp.bfloat16

B = 2
H = 32
S = 8192
DH = 128
DM = 512
DC = 512
BH = B * H

NSLOT = 3
CH = 128
NCH = S // CH
NSUB = 4
NTAIL = 4

NN = (((1,), (0,)), ((), ()))
NT = (((1,), (1,)), ((), ()))


def _dot(a, b, dims=NN):
    return lax.dot_general(a, b, dims, preferred_element_type=F32)


def _iota(shape, dim):
    return lax.broadcasted_iota(jnp.int32, shape, dim)


def _interleave(n, nsub=NSUB):
    return [(i % nsub) * (n // nsub) + i // nsub for i in range(n)]


def _kernel(xa_hbm, k_hbm, v_hbm, wq_hbm, wo_hbm,
            xb_hbm, ckv_hbm, wqb_hbm, wuk_hbm, wuv_hbm, wob_hbm,
            out_ref,
            xa_v, xb_v, wq_v, wo_v, ckv_v, wqb_v, wuk_v, wuv_v, wob_v,
            kbuf, vbuf, q_scr, e0_scr, acc_scr,
            wsem, ksem, vsem, tsem):
    SEM = dict(xa=0, xb=1, wq=2, wo=3, ckv0=4, ckv1=5, wqb=6, wuk=7, wuv=8, wob=9)

    def total(dst, sem):
        return pltpu.make_async_copy(dst, dst, sem)

    def wait_buf(name, dst):
        total(dst, wsem.at[SEM[name]]).wait()

    def row_chunks(name, src, dst, rows):
        n = dst.shape[0] // rows
        return [(src.at[pl.ds(c * rows, rows)], dst.at[pl.ds(c * rows, rows)],
                 wsem.at[SEM[name]]) for c in _interleave(n)]

    def wq_chunks():
        idx = [(pl.ds(16 * (c // 4), 16), pl.ds(1024 * (c % 4), 1024))
               for c in _interleave(128)]
        return [(wq_hbm.at[r, c], wq_v.at[r, c], wsem.at[SEM["wq"]]) for r, c in idx]

    def kv_chunk(src, buf, sem, i, slot, c):
        return (src.at[pl.ds(i * S + c * CH, CH)], buf.at[slot, pl.ds(c * CH, CH)], sem)

    def kv_pair(i, slot, t):
        c = _interleave(NCH)[t]
        return (kv_chunk(k_hbm, kbuf, ksem.at[slot], i, slot, c),
                kv_chunk(v_hbm, vbuf, vsem.at[slot], i, slot, c))

    def start_pair(pair):
        for prio, (src, dst, sem) in enumerate(pair):
            pltpu.make_async_copy(src, dst, sem).start(priority=prio)

    lane0 = (row_chunks("wqb", wqb_hbm, wqb_v, CH)
             + row_chunks("ckv0", ckv_hbm.at[0], ckv_v.at[0], 32)
             + row_chunks("wuv", wuv_hbm, wuv_v, CH)
             + wq_chunks())
    lane1 = (row_chunks("wuk", wuk_hbm, wuk_v, CH)
             + row_chunks("ckv1", ckv_hbm.at[1], ckv_v.at[1], 32)
             + row_chunks("wob", wob_hbm, wob_v, 32)
             + row_chunks("wo", wo_hbm, wo_v, 32))
    prologue = list(zip(lane0, lane1, strict=True))
    n_prefix = len(prologue)
    prologue += [kv_pair(0, 0, t) for t in range(NCH)]
    prologue += [kv_pair(1, 1, t) for t in range(NCH // 2)]
    issued = [0]
    AHEAD = 40

    def pump_to(n):
        n = min(n, len(prologue))
        while issued[0] < n:
            start_pair(prologue[issued[0]])
            issued[0] += 1

    def pump(n):
        pump_to(issued[0] + n)

    pltpu.make_async_copy(xa_hbm, xa_v, wsem.at[SEM["xa"]]).start()
    pltpu.make_async_copy(xb_hbm, xb_v, wsem.at[SEM["xb"]]).start()
    pump(32)

    for j in range(H // 8):
        w = 128 * 8
        e0_scr[:, j * w:(j + 1) * w] = (
            (_iota((128, w), 1) + j * w) // H == _iota((128, w), 0)).astype(BF16)
        pump(8)
    head_mask = (_iota((BH, 128), 1) % H) == (_iota((BH, 128), 0) % H)

    def mask_heads(t):
        return jnp.concatenate(
            [jnp.where(head_mask, t[:, j * 128:(j + 1) * 128], 0.0).astype(BF16)
             for j in range(t.shape[1] // 128)], axis=1)

    def expand_contract(lmat, w_ref):
        acc = jnp.zeros((BH, DH), F32)
        for u in range(lmat.shape[1] // 128):
            lx = mask_heads(_dot(lmat[:, u * 128:(u + 1) * 128], e0_scr[...]))
            acc = acc + _dot(lx, w_ref[pl.ds(u * 128 * H, 128 * H), :])
            pump(16)
        return acc

    def contract_compress(q, w_ref):
        outs = []
        for u in range(w_ref.shape[0] // (128 * H)):
            t = mask_heads(_dot(q, w_ref[pl.ds(u * 128 * H, 128 * H), :], NT))
            outs.append(_dot(t, e0_scr[...], NT))
            pump(16)
        return jnp.concatenate(outs, axis=1)

    pump_to(128 + AHEAD)
    wait_buf("xb", xb_v)
    wait_buf("wqb", wqb_v)
    wait_buf("wuk", wuk_v)
    xb = xb_v[...]
    xb_rows = jnp.concatenate(
        [jnp.broadcast_to(xb[b:b + 1, :], (H, DM)) for b in range(B)], axis=0)
    qb = expand_contract(xb_rows, wqb_v).astype(BF16)
    q_lat = contract_compress(qb, wuk_v).astype(BF16)

    pump_to(384 + AHEAD)
    NCKV = 4
    CKV = S // NCKV
    ctx_lat = []
    for b in range(B):
        wait_buf("ckv%d" % b, ckv_v.at[b])
        ql = q_lat[b * H:(b + 1) * H, :]
        ss = []
        for c in range(NCKV):
            ss.append(_dot(ql, ckv_v[b, pl.ds(c * CKV, CKV), :], NT))
            pump(8)
        s = jnp.concatenate(ss, axis=1) * (DH ** -0.5)
        m = jnp.max(s, axis=1, keepdims=True)
        p = jnp.exp(s - m)
        l = jnp.sum(p, axis=1, keepdims=True)
        pb = p.astype(BF16)
        pump(8)
        o = jnp.zeros((H, DC), F32)
        for c in range(NCKV):
            o = o + _dot(pb[:, c * CKV:(c + 1) * CKV], ckv_v[b, pl.ds(c * CKV, CKV), :])
            pump(8)
        ctx_lat.append(o / l)
    ctx_lat = jnp.concatenate(ctx_lat, axis=0).astype(BF16)

    pump_to(512 + AHEAD)
    wait_buf("wuv", wuv_v)
    ctx = expand_contract(ctx_lat, wuv_v).astype(BF16)
    ctx2 = jnp.concatenate(
        [jnp.concatenate([ctx[b * H + h:b * H + h + 1, :] for h in range(H)], axis=1)
         for b in range(B)] + [jnp.zeros((16 - B, H * DH), BF16)], axis=0)
    wait_buf("wob", wob_v)
    out_b = _dot(ctx2, wob_v[...])
    for b in range(B):
        out_ref[b:b + 1, DM:2 * DM] = out_b[b:b + 1, :].astype(out_ref.dtype)
    pump(16)

    pump_to(n_prefix + AHEAD)
    wait_buf("xa", xa_v)
    wait_buf("wq", wq_v)
    wait_buf("wo", wo_v)
    xa16 = jnp.concatenate([xa_v[...], jnp.zeros((16 - B, DM), BF16)], axis=0)
    qa = _dot(xa16, wq_v[...]).astype(BF16).astype(F32)
    for b in range(B):
        for h in range(H):
            q_scr[pl.ds(b * H + h, 1), :] = qa[b:b + 1, h * DH:(h + 1) * DH]
    acc_scr[...] = jnp.zeros_like(acc_scr)
    pump_to(len(prologue))

    def scores_softmax(i, slot):
        q = jnp.broadcast_to(q_scr[pl.ds(i, 1), :], (16, DH)).astype(BF16)
        s = _dot(q, kbuf[slot], NT)[0:8] * (DH ** -0.5)
        m = jnp.max(s, axis=1, keepdims=True)
        p = jnp.exp(s - m)
        l = jnp.sum(p, axis=1, keepdims=True)
        return jnp.concatenate([p, p], axis=0).astype(BF16), l

    def project(i, o, l):
        o = o[0:8] / l
        ob = jnp.concatenate([o, o], axis=0).astype(BF16)
        row = pl.multiple_of((i % H) * DH, DH)
        b = i // H
        acc_scr[b] = acc_scr[b] + _dot(ob, wo_v[pl.ds(row, DH), :])[0:8]

    def head_step(i, issue_a, issue_b):
        slot = i % NSLOT
        total(kbuf.at[slot], ksem.at[slot]).wait()
        total(vbuf.at[slot], vsem.at[slot]).wait()
        pb, l = scores_softmax(i, slot)
        issue_a()
        project(i, _dot(pb, vbuf[slot]), l)
        issue_b()

    def second_half(j):
        return lambda: [start_pair(kv_pair(j, j % NSLOT, t)) for t in range(NCH // 2, NCH)]

    def first_half(j):
        return lambda: [start_pair(kv_pair(j, j % NSLOT, t)) for t in range(NCH // 2)]

    def loop_body(i, carry):
        head_step(i, second_half(i + 1), first_half(i + 2))
        return carry

    last = BH - 1
    lslot = last % NSLOT

    def last_k():
        cs = _interleave(NCH, 2 * NSUB)
        for t in range(NCH // 2):
            start_pair([kv_chunk(k_hbm, kbuf, ksem.at[lslot], last, lslot, c)
                        for c in cs[2 * t:2 * t + 2]])

    def last_v():
        per = NCH // NTAIL
        for piece in range(NTAIL):
            cs = [piece * per + c for c in _interleave(per, 2 * NSUB)]
            for t in range(per // 2):
                start_pair([kv_chunk(v_hbm, vbuf, tsem.at[piece], last, lslot, c)
                            for c in cs[2 * t:2 * t + 2]])

    lax.fori_loop(0, BH - 3, loop_body, 0)
    head_step(BH - 3, second_half(BH - 2), last_k)
    head_step(BH - 2, last_v, lambda: None)

    total(kbuf.at[lslot], ksem.at[lslot]).wait()
    pb, l = scores_softmax(last, lslot)
    o = jnp.zeros((16, DH), F32)
    rows = S // NTAIL
    for piece in range(NTAIL):
        dst = vbuf.at[lslot, pl.ds(piece * rows, rows)]
        total(dst, tsem.at[piece]).wait()
        o = o + _dot(pb[:, piece * rows:(piece + 1) * rows], dst[...])
    project(last, o, l)

    for b in range(B):
        out_ref[b:b + 1, 0:DM] = acc_scr[b, 0:1, :].astype(out_ref.dtype)


@jax.jit
def pallas_concat_heads__gqa_block_cached__compressed_kv_cla__decode_kernel(
    A_x: jax.Array,
    A_k_cache: jax.Array,
    A_v_cache: jax.Array,
    A_wq: jax.Array,
    A_wo: jax.Array,
    B_x: jax.Array,
    B_c_kv: jax.Array,
    B_w_q: jax.Array,
    B_w_uk: jax.Array,
    B_w_uv: jax.Array,
    B_w_o: jax.Array,
):
    any_spec = pl.BlockSpec(memory_space=pl.ANY)
    scratch = [
        pltpu.VMEM((B, DM), BF16),
        pltpu.VMEM((B, DM), BF16),
        pltpu.VMEM((DM, H * DH), BF16),
        pltpu.VMEM((H * DH, DM), BF16),
        pltpu.VMEM((B, S, DC), BF16),
        pltpu.VMEM((DM * H, DH), BF16),
        pltpu.VMEM((DC * H, DH), BF16),
        pltpu.VMEM((DC * H, DH), BF16),
        pltpu.VMEM((H * DH, DM), BF16),
        pltpu.VMEM((NSLOT, S, DH), BF16),
        pltpu.VMEM((NSLOT, S, DH), BF16),
        pltpu.VMEM((BH, DH), F32),
        pltpu.VMEM((128, 128 * H), BF16),
        pltpu.VMEM((B, 8, DM), F32),
        pltpu.SemaphoreType.DMA((10,)),
        pltpu.SemaphoreType.DMA((NSLOT,)),
        pltpu.SemaphoreType.DMA((NSLOT,)),
        pltpu.SemaphoreType.DMA((NTAIL,)),
    ]
    out = pl.pallas_call(
        _kernel,
        out_shape=jax.ShapeDtypeStruct((B, 2 * DM), BF16),
        in_specs=[any_spec] * 11,
        out_specs=pl.BlockSpec(memory_space=pltpu.VMEM),
        scratch_shapes=scratch,
        compiler_params=pltpu.CompilerParams(vmem_limit_bytes=100 * 1024 * 1024),
    )(
        A_x.reshape(B, DM),
        A_k_cache.reshape(B * H * S, DH),
        A_v_cache.reshape(B * H * S, DH),
        A_wq,
        A_wo,
        B_x.reshape(B, DM),
        B_c_kv,
        B_w_q.reshape(DM * H, DH),
        B_w_uk.reshape(DC * H, DH),
        B_w_uv.reshape(DC * H, DH),
        B_w_o.reshape(H * DH, DM),
    )
    return out.reshape(B, 1, 2 * DM)
```

```python
import jax
import jax.numpy as jnp
from jax import lax
import jax.experimental.pallas as pl
import jax.experimental.pallas.tpu as pltpu

F32 = jnp.float32
BF16 = jnp.bfloat16

B = 2
H = 32
S = 8192
DH = 128
DM = 512
DC = 512
BH = B * H

NSLOT = 3
CH = 128
NCH = S // CH
NSUB = 4
NTAIL = 4

NN = (((1,), (0,)), ((), ()))
NT = (((1,), (1,)), ((), ()))


def _dot(a, b, dims=NN):
    return lax.dot_general(a, b, dims, preferred_element_type=F32)


def _iota(shape, dim):
    return lax.broadcasted_iota(jnp.int32, shape, dim)


def _interleave(n, nsub=NSUB):
    return [(i % nsub) * (n // nsub) + i // nsub for i in range(n)]


def _kernel(xa_hbm, k_hbm, v_hbm, wq_hbm, wo_hbm,
            xb_hbm, ckv_hbm, wqb_hbm, wuk_hbm, wuv_hbm, wob_hbm,
            out_ref,
            xa_v, xb_v, wq_v, wo_v, ckv_v, wqb_v, wuk_v, wuv_v, wob_v,
            kbuf, vbuf, q_scr, e0_scr, acc_scr,
            wsem, ksem, vsem, tsem, bsem):
    SEM = dict(xa=0, xb=1, wq=2, wo=3, ckv0=4, ckv1=5, wqb=6, wuk=7, wuv=8, wob=9)

    def total(dst, sem):
        return pltpu.make_async_copy(dst, dst, sem)

    def wait_buf(name, dst):
        total(dst, wsem.at[SEM[name]]).wait()

    def row_chunks(name, src, dst, rows):
        n = dst.shape[0] // rows
        return [(src.at[pl.ds(c * rows, rows)], dst.at[pl.ds(c * rows, rows)],
                 wsem.at[SEM[name]]) for c in _interleave(n)]

    def wq_chunks():
        idx = [(pl.ds(16 * (c // 4), 16), pl.ds(1024 * (c % 4), 1024))
               for c in _interleave(128)]
        return [(wq_hbm.at[r, c], wq_v.at[r, c], wsem.at[SEM["wq"]]) for r, c in idx]

    def kv_chunk(src, buf, sem, i, slot, c):
        return (src.at[pl.ds(i * S + c * CH, CH)], buf.at[slot, pl.ds(c * CH, CH)], sem)

    def kv_pair(i, slot, t):
        c = _interleave(NCH)[t]
        return (kv_chunk(k_hbm, kbuf, ksem.at[slot], i, slot, c),
                kv_chunk(v_hbm, vbuf, vsem.at[slot], i, slot, c))

    def start_pair(pair):
        for prio, (src, dst, sem) in enumerate(pair):
            pltpu.make_async_copy(src, dst, sem).start(priority=prio)

    lane0 = (row_chunks("wqb", wqb_hbm, wqb_v, CH)
             + row_chunks("ckv0", ckv_hbm.at[0], ckv_v.at[0], 32)
             + row_chunks("wuv", wuv_hbm, wuv_v, CH)
             + wq_chunks())
    lane1 = (row_chunks("wuk", wuk_hbm, wuk_v, CH)
             + row_chunks("ckv1", ckv_hbm.at[1], ckv_v.at[1], 32)
             + row_chunks("wob", wob_hbm, wob_v, 32)
             + row_chunks("wo", wo_hbm, wo_v, 32))
    prologue = list(zip(lane0, lane1, strict=True))
    n_prefix = len(prologue)
    prologue += [kv_pair(0, 0, t) for t in range(NCH)]
    prologue += [kv_pair(1, 1, t) for t in range(NCH // 2)]
    issued = [0]
    AHEAD = 40

    def pump_to(n):
        n = min(n, len(prologue))
        if issued[0] < n and issued[0] > 0:
            pl.semaphore_signal(bsem, 1)
            pl.semaphore_wait(bsem, 1)
        while issued[0] < n:
            start_pair(prologue[issued[0]])
            issued[0] += 1

    def pump(n):
        pump_to(issued[0] + n)

    pltpu.make_async_copy(xa_hbm, xa_v, wsem.at[SEM["xa"]]).start()
    pltpu.make_async_copy(xb_hbm, xb_v, wsem.at[SEM["xb"]]).start()
    pump(32)

    for j in range(H // 8):
        w = 128 * 8
        e0_scr[:, j * w:(j + 1) * w] = (
            (_iota((128, w), 1) + j * w) // H == _iota((128, w), 0)).astype(BF16)
        pump(8)
    head_mask = (_iota((BH, 128), 1) % H) == (_iota((BH, 128), 0) % H)

    def mask_heads(t):
        return jnp.concatenate(
            [jnp.where(head_mask, t[:, j * 128:(j + 1) * 128], 0.0).astype(BF16)
             for j in range(t.shape[1] // 128)], axis=1)

    def expand_contract(lmat, w_ref):
        acc = jnp.zeros((BH, DH), F32)
        for u in range(lmat.shape[1] // 128):
            lx = mask_heads(_dot(lmat[:, u * 128:(u + 1) * 128], e0_scr[...]))
            acc = acc + _dot(lx, w_ref[pl.ds(u * 128 * H, 128 * H), :])
            pump(16)
        return acc

    def contract_compress(q, w_ref):
        outs = []
        for u in range(w_ref.shape[0] // (128 * H)):
            t = mask_heads(_dot(q, w_ref[pl.ds(u * 128 * H, 128 * H), :], NT))
            outs.append(_dot(t, e0_scr[...], NT))
            pump(16)
        return jnp.concatenate(outs, axis=1)

    pump_to(128 + AHEAD)
    wait_buf("xb", xb_v)
    wait_buf("wqb", wqb_v)
    wait_buf("wuk", wuk_v)
    xb = xb_v[...]
    xb_rows = jnp.concatenate(
        [jnp.broadcast_to(xb[b:b + 1, :], (H, DM)) for b in range(B)], axis=0)
    qb = expand_contract(xb_rows, wqb_v).astype(BF16)
    q_lat = contract_compress(qb, wuk_v).astype(BF16)

    pump_to(384 + AHEAD)
    NCKV = 4
    CKV = S // NCKV
    ctx_lat = []
    for b in range(B):
        wait_buf("ckv%d" % b, ckv_v.at[b])
        ql = q_lat[b * H:(b + 1) * H, :]
        ss = []
        for c in range(NCKV):
            ss.append(_dot(ql, ckv_v[b, pl.ds(c * CKV, CKV), :], NT))
            pump(8)
        s = jnp.concatenate(ss, axis=1) * (DH ** -0.5)
        m = jnp.max(s, axis=1, keepdims=True)
        p = jnp.exp(s - m)
        l = jnp.sum(p, axis=1, keepdims=True)
        pb = p.astype(BF16)
        pump(8)
        o = jnp.zeros((H, DC), F32)
        for c in range(NCKV):
            o = o + _dot(pb[:, c * CKV:(c + 1) * CKV], ckv_v[b, pl.ds(c * CKV, CKV), :])
            pump(8)
        ctx_lat.append(o / l)
    ctx_lat = jnp.concatenate(ctx_lat, axis=0).astype(BF16)

    pump_to(512 + AHEAD)
    wait_buf("wuv", wuv_v)
    ctx = expand_contract(ctx_lat, wuv_v).astype(BF16)
    ctx2 = jnp.concatenate(
        [jnp.concatenate([ctx[b * H + h:b * H + h + 1, :] for h in range(H)], axis=1)
         for b in range(B)] + [jnp.zeros((16 - B, H * DH), BF16)], axis=0)
    wait_buf("wob", wob_v)
    out_b = _dot(ctx2, wob_v[...])
    for b in range(B):
        out_ref[b:b + 1, DM:2 * DM] = out_b[b:b + 1, :].astype(out_ref.dtype)
    pump(16)

    pump_to(n_prefix + AHEAD)
    wait_buf("xa", xa_v)
    wait_buf("wq", wq_v)
    wait_buf("wo", wo_v)
    xa16 = jnp.concatenate([xa_v[...], jnp.zeros((16 - B, DM), BF16)], axis=0)
    qa = _dot(xa16, wq_v[...]).astype(BF16).astype(F32)
    for b in range(B):
        for h in range(H):
            q_scr[pl.ds(b * H + h, 1), :] = qa[b:b + 1, h * DH:(h + 1) * DH]
    acc_scr[...] = jnp.zeros_like(acc_scr)
    pump_to(len(prologue))

    def scores_softmax(i, slot):
        q = jnp.broadcast_to(q_scr[pl.ds(i, 1), :], (16, DH)).astype(BF16)
        s = _dot(q, kbuf[slot], NT)[0:8] * (DH ** -0.5)
        m = jnp.max(s, axis=1, keepdims=True)
        p = jnp.exp(s - m)
        l = jnp.sum(p, axis=1, keepdims=True)
        return jnp.concatenate([p, p], axis=0).astype(BF16), l

    def project(i, o, l):
        o = o[0:8] / l
        ob = jnp.concatenate([o, o], axis=0).astype(BF16)
        row = pl.multiple_of((i % H) * DH, DH)
        b = i // H
        acc_scr[b] = acc_scr[b] + _dot(ob, wo_v[pl.ds(row, DH), :])[0:8]

    def head_step(i, issue_a, issue_b):
        slot = i % NSLOT
        total(kbuf.at[slot], ksem.at[slot]).wait()
        total(vbuf.at[slot], vsem.at[slot]).wait()
        pb, l = scores_softmax(i, slot)
        issue_a()
        project(i, _dot(pb, vbuf[slot]), l)
        issue_b()

    def second_half(j):
        return lambda: [start_pair(kv_pair(j, j % NSLOT, t)) for t in range(NCH // 2, NCH)]

    def first_half(j):
        return lambda: [start_pair(kv_pair(j, j % NSLOT, t)) for t in range(NCH // 2)]

    def loop_body(i, carry):
        head_step(i, second_half(i + 1), first_half(i + 2))
        return carry

    last = BH - 1
    lslot = last % NSLOT

    def last_k():
        cs = _interleave(NCH, 2 * NSUB)
        for t in range(NCH // 2):
            start_pair([kv_chunk(k_hbm, kbuf, ksem.at[lslot], last, lslot, c)
                        for c in cs[2 * t:2 * t + 2]])

    def last_v():
        per = NCH // NTAIL
        for piece in range(NTAIL):
            cs = [piece * per + c for c in _interleave(per, 2 * NSUB)]
            for t in range(per // 2):
                start_pair([kv_chunk(v_hbm, vbuf, tsem.at[piece], last, lslot, c)
                            for c in cs[2 * t:2 * t + 2]])

    lax.fori_loop(0, BH - 3, loop_body, 0)
    head_step(BH - 3, second_half(BH - 2), last_k)
    head_step(BH - 2, last_v, lambda: None)

    total(kbuf.at[lslot], ksem.at[lslot]).wait()
    pb, l = scores_softmax(last, lslot)
    o = jnp.zeros((16, DH), F32)
    rows = S // NTAIL
    for piece in range(NTAIL):
        dst = vbuf.at[lslot, pl.ds(piece * rows, rows)]
        total(dst, tsem.at[piece]).wait()
        o = o + _dot(pb[:, piece * rows:(piece + 1) * rows], dst[...])
    project(last, o, l)

    for b in range(B):
        out_ref[b:b + 1, 0:DM] = acc_scr[b, 0:1, :].astype(out_ref.dtype)


@jax.jit
def pallas_concat_heads__gqa_block_cached__compressed_kv_cla__decode_kernel(
    A_x: jax.Array,
    A_k_cache: jax.Array,
    A_v_cache: jax.Array,
    A_wq: jax.Array,
    A_wo: jax.Array,
    B_x: jax.Array,
    B_c_kv: jax.Array,
    B_w_q: jax.Array,
    B_w_uk: jax.Array,
    B_w_uv: jax.Array,
    B_w_o: jax.Array,
):
    any_spec = pl.BlockSpec(memory_space=pl.ANY)
    scratch = [
        pltpu.VMEM((B, DM), BF16),
        pltpu.VMEM((B, DM), BF16),
        pltpu.VMEM((DM, H * DH), BF16),
        pltpu.VMEM((H * DH, DM), BF16),
        pltpu.VMEM((B, S, DC), BF16),
        pltpu.VMEM((DM * H, DH), BF16),
        pltpu.VMEM((DC * H, DH), BF16),
        pltpu.VMEM((DC * H, DH), BF16),
        pltpu.VMEM((H * DH, DM), BF16),
        pltpu.VMEM((NSLOT, S, DH), BF16),
        pltpu.VMEM((NSLOT, S, DH), BF16),
        pltpu.VMEM((BH, DH), F32),
        pltpu.VMEM((128, 128 * H), BF16),
        pltpu.VMEM((B, 8, DM), F32),
        pltpu.SemaphoreType.DMA((10,)),
        pltpu.SemaphoreType.DMA((NSLOT,)),
        pltpu.SemaphoreType.DMA((NSLOT,)),
        pltpu.SemaphoreType.DMA((NTAIL,)),
        pltpu.SemaphoreType.REGULAR,
    ]
    out = pl.pallas_call(
        _kernel,
        out_shape=jax.ShapeDtypeStruct((B, 2 * DM), BF16),
        in_specs=[any_spec] * 11,
        out_specs=pl.BlockSpec(memory_space=pltpu.VMEM),
        scratch_shapes=scratch,
        compiler_params=pltpu.CompilerParams(vmem_limit_bytes=100 * 1024 * 1024, disable_bounds_checks=True),
    )(
        A_x.reshape(B, DM),
        A_k_cache.reshape(B * H * S, DH),
        A_v_cache.reshape(B * H * S, DH),
        A_wq,
        A_wo,
        B_x.reshape(B, DM),
        B_c_kv,
        B_w_q.reshape(DM * H, DH),
        B_w_uk.reshape(DC * H, DH),
        B_w_uv.reshape(DC * H, DH),
        B_w_o.reshape(H * DH, DM),
    )
    return out.reshape(B, 1, 2 * DM)
```

```python
import jax
import jax.numpy as jnp
from jax import lax
import jax.experimental.pallas as pl
import jax.experimental.pallas.tpu as pltpu

F32 = jnp.float32
BF16 = jnp.bfloat16

B = 2
H = 32
S = 8192
DH = 128
DM = 512
DC = 512
BH = B * H

NSLOT = 3
CH = 128
NCH = S // CH
NSUB = 4
NTAIL = 4

NN = (((1,), (0,)), ((), ()))
NT = (((1,), (1,)), ((), ()))


def _dot(a, b, dims=NN):
    return lax.dot_general(a, b, dims, preferred_element_type=F32)


def _iota(shape, dim):
    return lax.broadcasted_iota(jnp.int32, shape, dim)


def _interleave(n, nsub=NSUB):
    return [(i % nsub) * (n // nsub) + i // nsub for i in range(n)]


def _kernel(xa_hbm, k_hbm, v_hbm, wq_hbm, wo_hbm,
            xb_hbm, ckv_hbm, wqb_hbm, wuk_hbm, wuv_hbm, wob_hbm,
            out_ref,
            xa_v, xb_v, wq_v, wo_v, ckv_v, wqb_v, wuk_v, wuv_v, wob_v,
            kbuf, vbuf, q_scr, e0_scr, acc_scr,
            wsem, ksem, vsem, tsem, bsem):
    SEM = dict(xa=0, xb=1, wq=2, wo=3, ckv0=4, ckv1=5, wqb=6, wuk=7, wuv=8, wob=9)

    def total(dst, sem):
        return pltpu.make_async_copy(dst, dst, sem)

    def wait_buf(name, dst):
        total(dst, wsem.at[SEM[name]]).wait()

    def row_chunks(name, src, dst, rows):
        n = dst.shape[0] // rows
        return [(src.at[pl.ds(c * rows, rows)], dst.at[pl.ds(c * rows, rows)],
                 wsem.at[SEM[name]]) for c in _interleave(n)]

    def wq_chunks():
        idx = [(pl.ds(8 * (c // 2), 8), pl.ds(2048 * (c % 2), 2048))
               for c in _interleave(128)]
        return [(wq_hbm.at[r, c], wq_v.at[r, c], wsem.at[SEM["wq"]]) for r, c in idx]

    def kv_chunk(src, buf, sem, i, slot, c):
        return (src.at[pl.ds(i * S + c * CH, CH)], buf.at[slot, pl.ds(c * CH, CH)], sem)

    def kv_pair(i, slot, t):
        c = _interleave(NCH)[t]
        return (kv_chunk(k_hbm, kbuf, ksem.at[slot], i, slot, c),
                kv_chunk(v_hbm, vbuf, vsem.at[slot], i, slot, c))

    def start_pair(pair):
        for prio, (src, dst, sem) in enumerate(pair):
            pltpu.make_async_copy(src, dst, sem).start(priority=prio)

    lane0 = (row_chunks("wqb", wqb_hbm, wqb_v, CH)
             + row_chunks("ckv0", ckv_hbm.at[0], ckv_v.at[0], 32)
             + row_chunks("wuv", wuv_hbm, wuv_v, CH)
             + wq_chunks())
    lane1 = (row_chunks("wuk", wuk_hbm, wuk_v, CH)
             + row_chunks("ckv1", ckv_hbm.at[1], ckv_v.at[1], 32)
             + row_chunks("wob", wob_hbm, wob_v, 32)
             + row_chunks("wo", wo_hbm, wo_v, 32))
    prologue = list(zip(lane0, lane1, strict=True))
    n_prefix = len(prologue)
    prologue += [kv_pair(0, 0, t) for t in range(NCH)]
    prologue += [kv_pair(1, 1, t) for t in range(NCH)]
    issued = [0]
    AHEAD = 56

    def fence():
        pl.semaphore_signal(bsem, 1)
        pl.semaphore_wait(bsem, 1)

    def pump_to(n):
        n = min(n, len(prologue))
        if issued[0] < n and issued[0] > 0:
            fence()
        while issued[0] < n:
            start_pair(prologue[issued[0]])
            issued[0] += 1

    def pump(n):
        pump_to(issued[0] + n)

    pltpu.make_async_copy(xa_hbm, xa_v, wsem.at[SEM["xa"]]).start()
    pltpu.make_async_copy(xb_hbm, xb_v, wsem.at[SEM["xb"]]).start()
    pump(32)

    for j in range(H // 8):
        w = 128 * 8
        e0_scr[:, j * w:(j + 1) * w] = (
            (_iota((128, w), 1) + j * w) // H == _iota((128, w), 0)).astype(BF16)
        pump(8)
    head_mask = (_iota((BH, 128), 1) % H) == (_iota((BH, 128), 0) % H)

    def mask_heads(t):
        return jnp.concatenate(
            [jnp.where(head_mask, t[:, j * 128:(j + 1) * 128], 0.0).astype(BF16)
             for j in range(t.shape[1] // 128)], axis=1)

    def expand_contract(lmat, w_ref):
        acc = jnp.zeros((BH, DH), F32)
        for u in range(lmat.shape[1] // 128):
            lx = mask_heads(_dot(lmat[:, u * 128:(u + 1) * 128], e0_scr[...]))
            acc = acc + _dot(lx, w_ref[pl.ds(u * 128 * H, 128 * H), :])
            pump(16)
        return acc

    def contract_compress(q, w_ref):
        outs = []
        for u in range(w_ref.shape[0] // (128 * H)):
            t = mask_heads(_dot(q, w_ref[pl.ds(u * 128 * H, 128 * H), :], NT))
            outs.append(_dot(t, e0_scr[...], NT))
            pump(16)
        return jnp.concatenate(outs, axis=1)

    pump_to(128 + AHEAD)
    wait_buf("xb", xb_v)
    wait_buf("wqb", wqb_v)
    wait_buf("wuk", wuk_v)
    xb = xb_v[...]
    xb_rows = jnp.concatenate(
        [jnp.broadcast_to(xb[b:b + 1, :], (H, DM)) for b in range(B)], axis=0)
    qb = expand_contract(xb_rows, wqb_v).astype(BF16)
    q_lat = contract_compress(qb, wuk_v).astype(BF16)

    pump_to(384 + AHEAD)
    NCKV = 4
    CKV = S // NCKV
    ctx_lat = []
    for b in range(B):
        wait_buf("ckv%d" % b, ckv_v.at[b])
        ql = q_lat[b * H:(b + 1) * H, :]
        ss = []
        for c in range(NCKV):
            ss.append(_dot(ql, ckv_v[b, pl.ds(c * CKV, CKV), :], NT))
            pump(8)
        s = jnp.concatenate(ss, axis=1) * (DH ** -0.5)
        m = jnp.max(s, axis=1, keepdims=True)
        p = jnp.exp(s - m)
        l = jnp.sum(p, axis=1, keepdims=True)
        pb = p.astype(BF16)
        pump(8)
        o = jnp.zeros((H, DC), F32)
        for c in range(NCKV):
            o = o + _dot(pb[:, c * CKV:(c + 1) * CKV], ckv_v[b, pl.ds(c * CKV, CKV), :])
            pump(8)
        ctx_lat.append(o / l)
    ctx_lat = jnp.concatenate(ctx_lat, axis=0).astype(BF16)

    pump_to(512 + AHEAD)
    wait_buf("wuv", wuv_v)
    ctx = expand_contract(ctx_lat, wuv_v).astype(BF16)
    ctx2 = jnp.concatenate(
        [jnp.concatenate([ctx[b * H + h:b * H + h + 1, :] for h in range(H)], axis=1)
         for b in range(B)] + [jnp.zeros((16 - B, H * DH), BF16)], axis=0)
    wait_buf("wob", wob_v)
    out_b = _dot(ctx2, wob_v[...])
    for b in range(B):
        out_ref[b:b + 1, DM:2 * DM] = out_b[b:b + 1, :].astype(out_ref.dtype)
    pump(16)

    pump_to(n_prefix + AHEAD)
    wait_buf("xa", xa_v)
    wait_buf("wq", wq_v)
    wait_buf("wo", wo_v)
    xa16 = jnp.concatenate([xa_v[...], jnp.zeros((16 - B, DM), BF16)], axis=0)
    qa = _dot(xa16, wq_v[...]).astype(BF16).astype(F32)
    for b in range(B):
        for h in range(H):
            q_scr[pl.ds(b * H + h, 1), :] = qa[b:b + 1, h * DH:(h + 1) * DH]
    acc_scr[...] = jnp.zeros_like(acc_scr)
    pump_to(len(prologue))

    def scores_softmax(i, slot):
        q = jnp.broadcast_to(q_scr[pl.ds(i, 1), :], (16, DH)).astype(BF16)
        s = _dot(q, kbuf[slot], NT)[0:8] * (DH ** -0.5)
        m = jnp.max(s, axis=1, keepdims=True)
        p = jnp.exp(s - m)
        l = jnp.sum(p, axis=1, keepdims=True)
        return jnp.concatenate([p, p], axis=0).astype(BF16), l

    def project(i, o, l):
        o = o[0:8] / l
        ob = jnp.concatenate([o, o], axis=0).astype(BF16)
        row = pl.multiple_of((i % H) * DH, DH)
        b = i // H
        acc_scr[b] = acc_scr[b] + _dot(ob, wo_v[pl.ds(row, DH), :])[0:8]

    def head_step(i, issue):
        slot = i % NSLOT
        total(kbuf.at[slot], ksem.at[slot]).wait()
        total(vbuf.at[slot], vsem.at[slot]).wait()
        pb, l = scores_softmax(i, slot)
        project(i, _dot(pb, vbuf[slot]), l)
        issue()

    def issue_head(j):
        for t in range(NCH):
            start_pair(kv_pair(j, j % NSLOT, t))

    def loop_body(i, carry):
        head_step(i, lambda: issue_head(i + 2))
        return carry

    last = BH - 1
    lslot = last % NSLOT

    def last_k():
        cs = _interleave(NCH, 2 * NSUB)
        for t in range(NCH // 2):
            start_pair([kv_chunk(k_hbm, kbuf, ksem.at[lslot], last, lslot, c)
                        for c in cs[2 * t:2 * t + 2]])

    def last_v():
        per = NCH // NTAIL
        for piece in range(NTAIL):
            cs = [piece * per + c for c in _interleave(per, 2 * NSUB)]
            for t in range(per // 2):
                start_pair([kv_chunk(v_hbm, vbuf, tsem.at[piece], last, lslot, c)
                            for c in cs[2 * t:2 * t + 2]])

    lax.fori_loop(0, BH - 3, loop_body, 0)
    head_step(BH - 3, last_k)
    head_step(BH - 2, last_v)

    total(kbuf.at[lslot], ksem.at[lslot]).wait()
    pb, l = scores_softmax(last, lslot)
    o = jnp.zeros((16, DH), F32)
    rows = S // NTAIL
    for piece in range(NTAIL):
        dst = vbuf.at[lslot, pl.ds(piece * rows, rows)]
        total(dst, tsem.at[piece]).wait()
        o = o + _dot(pb[:, piece * rows:(piece + 1) * rows], dst[...])
    project(last, o, l)

    for b in range(B):
        out_ref[b:b + 1, 0:DM] = acc_scr[b, 0:1, :].astype(out_ref.dtype)


@jax.jit
def pallas_concat_heads__gqa_block_cached__compressed_kv_cla__decode_kernel(
    A_x: jax.Array,
    A_k_cache: jax.Array,
    A_v_cache: jax.Array,
    A_wq: jax.Array,
    A_wo: jax.Array,
    B_x: jax.Array,
    B_c_kv: jax.Array,
    B_w_q: jax.Array,
    B_w_uk: jax.Array,
    B_w_uv: jax.Array,
    B_w_o: jax.Array,
):
    any_spec = pl.BlockSpec(memory_space=pl.ANY)
    scratch = [
        pltpu.VMEM((B, DM), BF16),
        pltpu.VMEM((B, DM), BF16),
        pltpu.VMEM((DM, H * DH), BF16),
        pltpu.VMEM((H * DH, DM), BF16),
        pltpu.VMEM((B, S, DC), BF16),
        pltpu.VMEM((DM * H, DH), BF16),
        pltpu.VMEM((DC * H, DH), BF16),
        pltpu.VMEM((DC * H, DH), BF16),
        pltpu.VMEM((H * DH, DM), BF16),
        pltpu.VMEM((NSLOT, S, DH), BF16),
        pltpu.VMEM((NSLOT, S, DH), BF16),
        pltpu.VMEM((BH, DH), F32),
        pltpu.VMEM((128, 128 * H), BF16),
        pltpu.VMEM((B, 8, DM), F32),
        pltpu.SemaphoreType.DMA((10,)),
        pltpu.SemaphoreType.DMA((NSLOT,)),
        pltpu.SemaphoreType.DMA((NSLOT,)),
        pltpu.SemaphoreType.DMA((NTAIL,)),
        pltpu.SemaphoreType.REGULAR,
    ]
    out = pl.pallas_call(
        _kernel,
        out_shape=jax.ShapeDtypeStruct((B, 2 * DM), BF16),
        in_specs=[any_spec] * 11,
        out_specs=pl.BlockSpec(memory_space=pltpu.VMEM),
        scratch_shapes=scratch,
        compiler_params=pltpu.CompilerParams(vmem_limit_bytes=100 * 1024 * 1024),
    )(
        A_x.reshape(B, DM),
        A_k_cache.reshape(B * H * S, DH),
        A_v_cache.reshape(B * H * S, DH),
        A_wq,
        A_wo,
        B_x.reshape(B, DM),
        B_c_kv,
        B_w_q.reshape(DM * H, DH),
        B_w_uk.reshape(DC * H, DH),
        B_w_uv.reshape(DC * H, DH),
        B_w_o.reshape(H * DH, DM),
    )
    return out.reshape(B, 1, 2 * DM)
```
